```python
import jax
import jax.numpy as jnp

def _softmax(x, axis=-1):
    return jax.nn.softmax(x, axis=axis)
def _gelu(x):
    return jax.nn.gelu(x, approximate=True)
def _silu(x):
    return jax.nn.silu(x)
def _sigmoid(x):
    return jax.nn.sigmoid(x)
def _layernorm(x, axis=-1, eps=1e-5):
    m = jnp.mean(x, axis=axis, keepdims=True)
    v = jnp.var(x, axis=axis, keepdims=True)
    return (x - m) / jnp.sqrt(v + eps)
def _scatter_add(tgt, idx, src, axis=0):
    return tgt.at[idx].add(src)
def _segment_sum(src, seg, n):
    return jax.ops.segment_sum(src, seg, n)
class _Rng:
    def __init__(self, key):
        self._k = key
    def _next(self):
        self._k, sub = jax.random.split(self._k)
        return sub
    def normal(self, shape):
        return jax.random.normal(self._next(), shape, dtype=jnp.bfloat16)
    def randint(self, lo, hi, shape):
        return jax.random.randint(self._next(), shape, lo, hi, dtype=jnp.int32)
    def uniform(self, shape, lo=0.0, hi=1.0):
        return jax.random.uniform(self._next(), shape, jnp.bfloat16, lo, hi)
    def permutation(self, n):
        return jax.random.permutation(self._next(), n)


kernel_name = 'recurrent_scan__sliding_block_cached__moe_arch_mod__decode'

def setup_inputs():
    _rng = _Rng(jax.random.key(int.from_bytes(__import__("os").urandom(4), "little")))
    _w = (lambda a: (lambda t: t.astype(jnp.bfloat16) if jnp.issubdtype(t.dtype, jnp.floating) else t)(jnp.asarray(a)))
    def _A_setup():
        B, Sq, D = 1, 1, 512
        Hq, Hkv, Sk, Dh = 32, 32, 32768, 128
        assert Hq % Hkv == 0, (Hq, Hkv)
        return {
            "x": _w((lambda *s: _rng.normal(s) * 0.05)(B, Sq, D)),
            "k_cache": _w((lambda *s: _rng.normal(s) * 0.05)(B, Hkv, Sk, Dh)),
            "v_cache": _w((lambda *s: _rng.normal(s) * 0.05)(B, Hkv, Sk, Dh)),
            "wq": _w((lambda *s: _rng.normal(s) * 0.05)(D, Hq * Dh) * (D ** -0.5)),
            "wo": _w((lambda *s: _rng.normal(s) * 0.05)(Hq * Dh, D) * ((Hq * Dh) ** -0.5)),
        }
    _A_in = _A_setup()

    def _B_setup():
        B, S, D, F, C = 1, 1, 512, 1376, 1
        return {
            "x": _w((lambda *s: _rng.normal(s) * 0.05)(B, S, D)),
            "w_r": _w((lambda *s: _rng.normal(s) * 0.05)(D)),
            "w_gate": _w((lambda *s: _rng.normal(s) * 0.05)(D, F)),
            "w_up": _w((lambda *s: _rng.normal(s) * 0.05)(D, F)),
            "w_down": _w((lambda *s: _rng.normal(s) * 0.05)(F, D)),
        }
    _B_in = _B_setup()

    return {
        "A_x": _A_in["x"],
        "A_k_cache": _A_in["k_cache"],
        "A_v_cache": _A_in["v_cache"],
        "A_wq": _A_in["wq"],
        "A_wo": _A_in["wo"],
        "B_x": _B_in["x"],
        "B_w_r": _B_in["w_r"],
        "B_w_gate": _B_in["w_gate"],
        "B_w_up": _B_in["w_up"],
        "B_w_down": _B_in["w_down"],
    }

def reference(A_x, A_k_cache, A_v_cache, A_wq, A_wo, B_x, B_w_r, B_w_gate, B_w_up, B_w_down):
    def _A_ref(x, k_cache, v_cache, wq, wo):
        B, Sq, D = x.shape
        Hq, Dh = 32, 128
        Hkv, Sk = k_cache.shape[1], k_cache.shape[2]
        W = min(4096, max(256, Sk // 4))
        rep = Hq // Hkv
        q = (lambda x, *d: x.transpose(*d))((x @ wq).reshape(B, Sq, Hq, Dh), 0, 2, 1, 3)
        k = jnp.repeat(k_cache[:, :, Sk - W:, :], rep, axis=1)
        v = jnp.repeat(v_cache[:, :, Sk - W:, :], rep, axis=1)
        scores = jnp.einsum("bhqd,bhkd->bhqk", q, k) * (Dh ** -0.5)
        p = _softmax(scores, axis=-1)
        o = jnp.einsum("bhqk,bhkd->bhqd", p, v)
        return (lambda x, *d: x.transpose(*d))(o, 0, 2, 1, 3).reshape(B, Sq, Hq * Dh) @ wo

    def _B_ref(x, w_r, w_gate, w_up, w_down):
        B, S, D = x.shape
        C = 1
        r = x @ w_r
        idx = jnp.argsort(-r, axis=-1)[:, :C]
        idx_e = jnp.repeat(idx.reshape(B, C, 1), D, axis=2)
        x_sel = jnp.take_along_axis(x, idx_e, axis=1)
        g = _silu(x_sel @ w_gate)
        u = x_sel @ w_up
        y = (g * u) @ w_down
        r_sel = _sigmoid(jnp.take_along_axis(r, idx, axis=1))
        y = y * r_sel.reshape(B, C, 1)
        b_off = (jnp.arange(B) * S).reshape(B, 1)
        flat_idx = (idx + b_off).reshape(B * C)
        zero = (x * 0.0).reshape(B * S, D)
        upd = _scatter_add(zero, flat_idx, y.reshape(B * C, D), axis=0)
        return x + upd.reshape(B, S, D)

    x = A_x
    xn = _layernorm(x, axis=-1)
    s = _A_ref(xn, A_k_cache, A_v_cache, A_wq, A_wo)
    g = _silu(_B_ref(xn, B_w_r, B_w_gate, B_w_up, B_w_down))
    return x + s * g
```

```python
import jax
import jax.numpy as jnp
import jax.experimental.pallas as pl
import jax.experimental.pallas.tpu as pltpu

D = 512
NH = 32
DH = 128
SK = 32768
W = min(4096, max(256, SK // 4))
F = 1376

FH = F // 2
NB = W // DH
RUN = 64
NF = (5, 5, 6, 5, 5, 6, 5, 6)
NWB = len(NF)
LAG = 2
NSEM = LAG + 1
TAIL = (8, 8, 8, 8, 8, 8, 8, 4, 2, 1, 1)
T_BUSY, T_IDLE, T_FIRST = 46, 60, 50

BF16 = jnp.bfloat16
F32 = jnp.float32
_NT = (((1,), (1,)), ((), ()))
LONG, SHORT = 1, 0


def _rows(start, size, align):
    return pl.ds(start if isinstance(start, int) else pl.multiple_of(start, align), size)


def _per_head(f):
    r = f(0)
    for j in range(1, 8):
        r = jnp.where(jax.lax.broadcasted_iota(jnp.int32, r.shape, 0) == j, f(j), r)
    return r


def _kernel(x_h, k_h, v_h, wq_h, wo_h, wr_h, wg_h, wu_h, wd_h, out_ref,
            x_v, wr_v, wq_v, kv_v, wo_v, wf_v, q_v, s_v, m_v, l_v, o_v, c_v, y_v,
            sem_x, sem_long, sem_short, sem_tail):
    kv_h = (k_h, v_h)
    wf_h = (wg_h, wu_h, wd_h)
    everything = slice(None)

    def batch(i, longs, shorts, long_dst, short_dst):
        s_long, s_short = sem_long.at[i % NSEM], sem_short.at[i % NSEM]

        def wait():
            pltpu.make_async_copy(long_dst, long_dst, s_long).wait()
            pltpu.make_async_copy(short_dst, short_dst, s_short).wait()

        return (lambda: [pltpu.make_async_copy(a, b, s_long) for a, b in longs()],
                lambda: [pltpu.make_async_copy(a, b, s_short) for a, b in shorts()], wait)

    def weight_batch(b):
        cols = pl.ds((b // 2) * 8 * DH, 8 * DH)
        r0, f0 = (b % 2) * 32, 16 * sum(NF[:b])
        q_idx = [(everything, pl.ds(r0 + 8 * i, 8), cols) for i in range(4)]
        f_idx = [(everything, pl.ds(f0 + 16 * i, 16)) for i in range(NF[b])]
        return batch(b, lambda: [(wq_h.at[i], wq_v.at[i]) for i in q_idx],
                     lambda: [(wf_h[a].at[i], wf_v.at[(a,) + i]) for i in f_idx for a in range(3)],
                     wq_v.at[:, pl.ds(r0, 32), cols], wf_v.at[:, :, pl.ds(f0, 16 * NF[b])])

    def kv_batch(t, b):
        def part(h, n, r):
            return (kv_h[t].at[0, pl.ds(h, n), _rows(SK - W + r, RUN, RUN)],
                    kv_v.at[t, pl.ds(h, n), _rows(r, RUN, RUN)])

        h0, r0 = 16 + 8 * (b // 16), (b % 16) * 2 * DH
        return batch(NWB + t * NB + b, lambda: [part(0, 16, b * DH + i * RUN) for i in range(2)],
                     lambda: [part(h0 + 2 * (i % 4), 2, r0 + (i // 4) * RUN) for i in range(16)],
                     kv_v.at[t, pl.ds(0, 16), _rows(b * DH, DH, DH)],
                     kv_v.at[t, pl.ds(h0, 8), _rows(r0, 2 * DH, DH)])

    def wo_batch(b):
        def part(g, n, i):
            idx = (pl.ds(g, n), pl.ds(b * DH + 16 * i, 16))
            return wo_h.at[idx], wo_v.at[idx]

        return batch(NWB + 2 * NB + b, lambda: [part(0, 4, i) for i in range(8)],
                     lambda: [part(4 + 2 * (i % 2), 2, i // 2) for i in range(16)],
                     wo_v.at[pl.ds(0, 4), pl.ds(b * DH, DH)], wo_v.at[pl.ds(4, 4), pl.ds(b * DH, DH)])

    def step(landed, issue, work, pause, more_longs=()):
        if landed is not None:
            landed[2]()
        longs, shorts = (issue[0](), issue[1]()) if issue is not None else ([], [])
        for c in (*longs, *more_longs):
            c.start(priority=LONG)
        for i, c in enumerate(shorts):
            if i == 8:
                work()
            c.start(priority=SHORT)
            pl.delay(pause)
        if not shorts:
            work()

    tok = {}
    copy_x = pltpu.make_async_copy(x_h, x_v, sem_x.at[0])
    copy_wr = pltpu.make_async_copy(wr_h, wr_v, sem_x.at[1])

    def fetch_token():
        copy_x.start(priority=SHORT)
        copy_wr.start(priority=SHORT)

    def layernorm():
        copy_x.wait()
        copy_wr.wait()
        x = x_v[0].astype(F32)
        mean = jnp.mean(x, axis=-1, keepdims=True)
        var = jnp.mean(jnp.square(x - mean), axis=-1, keepdims=True)
        xn = ((x - mean) / jnp.sqrt(var + 1e-5)).astype(BF16)
        tok.update(x=x, xn=xn.astype(F32), xn8=jnp.broadcast_to(xn, (8, D)))
        tok["r"] = jnp.sum(tok["xn"] * wr_v[...].reshape(1, D).astype(F32), axis=-1, keepdims=True)
        m_v[...] = jnp.full(m_v.shape, -jnp.inf, F32)
        l_v[...] = jnp.zeros(l_v.shape, F32)
        o_v[...] = jnp.zeros(o_v.shape, F32)
        y_v[...] = jnp.zeros(y_v.shape, F32)

    def proj_q(s):
        w = wq_v[:, :, pl.ds(s * 8 * DH, 8 * DH)].reshape(D, 8 * DH)
        q = jnp.dot(tok["xn8"], w, preferred_element_type=F32)
        q_v[s] = _per_head(lambda j: q[:, j * DH:(j + 1) * DH])

    def ffn(r0, n):
        g, u, d = (wf_v[a, :, pl.ds(r0, n)].reshape(2 * n, D) for a in range(3))
        gt = jax.lax.dot_general(tok["xn8"], g, _NT, preferred_element_type=F32)
        up = jax.lax.dot_general(tok["xn8"], u, _NT, preferred_element_type=F32)
        y_v[...] += jnp.dot((jax.nn.silu(gt) * up).astype(BF16), d, preferred_element_type=F32)

    def tiles(b):
        return ((0, b, 1), (1, b, 1), (2 + b // 16, (b % 16) * 2, 2))

    def scores(b):
        for s, c, n in tiles(b):
            q = q_v[s].astype(BF16)
            sc = _per_head(lambda j: jax.lax.dot_general(
                q, kv_v[0, 8 * s + j, _rows(c * DH, n * DH, DH)], _NT, preferred_element_type=F32))
            sc = sc * (DH ** -0.5)
            m = m_v[s]
            for i in range(n):
                s_v[s, c + i] = sc[:, i * DH:(i + 1) * DH]
                m = jnp.maximum(m, sc[:, i * DH:(i + 1) * DH])
            m_v[s] = m

    def values(b):
        for s, c, n in tiles(b):
            ps = [jnp.exp(s_v[s, c + i] - m_v[s]) for i in range(n)]
            l_v[s] += sum(ps[1:], ps[0])
            p = jnp.concatenate(ps, axis=1).astype(BF16)
            o_v[s] += _per_head(lambda j: jnp.dot(
                p, kv_v[1, 8 * s + j, _rows(c * DH, n * DH, DH)], preferred_element_type=F32))

    def normalize():
        for s in range(NH // 8):
            o = o_v[s] / jnp.sum(l_v[s], axis=-1, keepdims=True)
            o_v[s] = o.astype(BF16).astype(F32)
        y_v[...] = jnp.zeros(y_v.shape, F32)

    def proj_o(b):
        row = jax.lax.broadcasted_iota(jnp.int32, (8, D), 0)
        acc = y_v[...]
        for g in range(8):
            t = jnp.dot(o_v[g // 2].astype(BF16), wo_v[g, pl.ds(b * DH, DH)], preferred_element_type=F32)
            acc = acc + jnp.where(row == 4 * (g % 2) + b, t, 0.0)
        y_v[...] = acc

    for i in range(NWB + LAG):
        done = i - LAG
        if i < 2:
            work, pause = (fetch_token, layernorm)[i], (T_FIRST, T_IDLE)[i]
        elif done % 2 == 1:
            work, pause = lambda: proj_q(done // 2), T_BUSY
        elif done >= 2:
            work, pause = lambda: ffn((done // 2 - 1) * 160, 160), T_BUSY
        else:
            work, pause = lambda: None, T_IDLE
        step(weight_batch(done) if done >= 0 else None,
             weight_batch(i) if i < NWB else kv_batch(0, i - NWB), work, pause)

    @pl.loop(LAG, NB)
    def _(b):
        step(kv_batch(0, b - LAG), kv_batch(0, b), lambda: scores(b - LAG), T_BUSY)

    @pl.loop(0, LAG)
    def _(b):
        step(kv_batch(0, NB - LAG + b), kv_batch(1, b), lambda: scores(NB - LAG + b), T_BUSY)

    for s in range(NH // 8):
        m_v[s] = jnp.broadcast_to(jnp.max(m_v[s], axis=-1, keepdims=True), (8, DH))
    ffn(480, FH - 480)
    upd = tok["xn"] * 0.0 + y_v[...] * jax.nn.sigmoid(tok["r"])
    gate = jax.nn.silu(tok["xn"] + upd)

    @pl.loop(LAG, NB)
    def _(b):
        step(kv_batch(1, b - LAG), kv_batch(1, b), lambda: values(b - LAG), T_BUSY)

    pieces, pos = [], 0
    for n in TAIL:
        idx = (pl.ds(pos % 8, n), pl.ds(3 * DH + (pos // 8) * 16, 16))
        pieces.append(pltpu.make_async_copy(wo_h.at[idx], wo_v.at[idx], sem_tail.at[len(pieces)]))
        pos += n

    assert LAG == 2 and pos == 64
    step(kv_batch(1, NB - 2), wo_batch(0), lambda: values(NB - 2), T_BUSY)
    step(kv_batch(1, NB - 1), wo_batch(1), lambda: (values(NB - 1), normalize()), T_BUSY)
    step(wo_batch(0), wo_batch(2), lambda: proj_o(0), T_BUSY, pieces)
    step(wo_batch(1), None, lambda: proj_o(1), T_BUSY)
    for g in range(8):
        j = 4 * (g % 2) + 3
        c_v[g] = jnp.broadcast_to(o_v[g // 2, j:j + 1], (DH, DH)).T
    step(wo_batch(2), None, lambda: proj_o(2), T_BUSY)

    part, pos = y_v[...], 0
    for n, c in zip(TAIL, pieces):
        c.wait()
        r0 = (pos // 8) * 16
        for g in range(pos % 8, pos % 8 + n):
            coef = jnp.concatenate([c_v[g, pl.ds(r0, 16)]] * (D // DH), axis=1)
            prod = wo_v[g, pl.ds(3 * DH + r0, 16)].astype(F32) * coef
            part = part + (prod[0:8] + prod[8:16])
        pos += n
    attn = jnp.sum(part, axis=0, keepdims=True)

    res = jnp.broadcast_to(tok["x"], (8, D)) + jnp.broadcast_to(attn, (8, D)) * gate
    out_ref[0] = res.astype(out_ref.dtype)[0:1]


@jax.jit
def pallas_recurrent_scan__sliding_block_cached__moe_arch_mod__decode_kernel(
    A_x: jax.Array,
    A_k_cache: jax.Array,
    A_v_cache: jax.Array,
    A_wq: jax.Array,
    A_wo: jax.Array,
    B_x: jax.Array,
    B_w_r: jax.Array,
    B_w_gate: jax.Array,
    B_w_up: jax.Array,
    B_w_down: jax.Array,
):
    del B_x
    hbm = pl.BlockSpec(memory_space=pltpu.HBM)
    dma = pltpu.SemaphoreType.DMA
    per_head = pltpu.VMEM((NH // 8, 8, DH), F32)
    return pl.pallas_call(
        _kernel,
        out_shape=jax.ShapeDtypeStruct((1, 1, D), BF16),
        in_specs=[hbm] * 9,
        out_specs=pl.BlockSpec(memory_space=pltpu.VMEM),
        scratch_shapes=[
            pltpu.VMEM((1, 1, D), BF16),
            pltpu.VMEM((D,), BF16),
            pltpu.VMEM((8, D // 8, NH * DH), BF16),
            pltpu.VMEM((2, NH, W, DH), BF16),
            pltpu.VMEM((8, NH * DH // 8, D), BF16),
            pltpu.VMEM((3, 2, FH, D), BF16),
            per_head,
            pltpu.VMEM((NH // 8, NB, 8, DH), F32),
            per_head, per_head, per_head,
            pltpu.VMEM((8, DH, DH), F32),
            pltpu.VMEM((8, D), F32),
            dma((2,)), dma((NSEM,)), dma((NSEM,)), dma((len(TAIL),)),
        ],
        compiler_params=pltpu.CompilerParams(
            vmem_limit_bytes=100 * 1024 * 1024,
            disable_semaphore_checks=True,
        ),
    )(A_x, A_k_cache, A_v_cache, A_wq.reshape(8, D // 8, NH * DH), A_wo.reshape(8, NH * DH // 8, D), B_w_r,
      B_w_gate.T.reshape(2, FH, D), B_w_up.T.reshape(2, FH, D), B_w_down.reshape(2, FH, D))
```

```python
import jax
import jax.numpy as jnp
import jax.experimental.pallas as pl
import jax.experimental.pallas.tpu as pltpu

D = 512
NH = 32
DH = 128
SK = 32768
W = min(4096, max(256, SK // 4))
F = 1376

NT = W // DH
NS = NH // 8
RUN = 64
EARLY = 16
FH = F // 2
F0, FB = 48, 80
NSEM = 3
HEADS_ALL = (((0, 11),), ((11, 11),), ((22, 10),))
HEADS_LONG = (((0, 10),), ((10, 10),))
HEADS_SHORT = (((20, 2), (22, 2), (24, 2)), ((26, 2), (28, 2), (30, 2)))
TAIL = (8, 8, 8, 8, 8, 8, 4, 2, 1, 1)
T_OPEN, T_FIRST, T_W, T_Q, T_F, T_K, T_V, T_VO, T_O = 27, 30, 54, 47, 50, 58, 50, 46, 54

BF16 = jnp.bfloat16
F32 = jnp.float32
_NT = (((1,), (1,)), ((), ()))
LONG, SHORT = 1, 0


def _rows(start, size, align):
    return pl.ds(start if isinstance(start, int) else pl.multiple_of(start, align), size)


def _per_head(f):
    r = f(0)
    for j in range(1, 8):
        r = jnp.where(jax.lax.broadcasted_iota(jnp.int32, r.shape, 0) == j, f(j), r)
    return r


def _kernel(x_h, k_h, v_h, wq_h, wo_h, wr_h, wg_h, wu_h, wd_h, out_ref,
            x_v, wr_v, wq_v, kv_v, wo_v, wf_v, q_v, s_v, m_v, l_v, o_v, c_v, g_v,
            sem_x, sem_long, sem_short, sem_tail):
    kv_h = (k_h, v_h)
    wf_h = (wg_h, wu_h, wd_h)

    def kv(t, j, heads):
        r = (2 * j - t) * RUN
        wraps = isinstance(r, int) and r < 0
        runs = (r + W if wraps else r, r + RUN)
        hs = pl.ds(heads[0][0][0], sum(n for group in heads for _, n in group))
        return (lambda: [(kv_h[t].at[0, pl.ds(h, n), _rows(SK - W + r, RUN, RUN)],
                          kv_v.at[t, pl.ds(h, n), _rows(r, RUN, RUN)])
                         for group in heads for r in runs for h, n in group],
                [kv_v.at[t, hs, pl.ds(r, RUN)] for r in runs] if wraps
                else [kv_v.at[t, hs, _rows(r, 2 * RUN, RUN)]])

    def wq(b):
        rows = _rows(8 * b, 8, 8)
        idx = [(g0 + g, rows, pl.ds((c0 + c) * 8 * DH, 8 * DH))
               for c0 in (0, 2) for g0 in (0, 4) for c in range(2) for g in range(4)]
        return lambda: [(wq_h.at[i], wq_v.at[i]) for i in idx], [wq_v.at[:, rows]]

    def wf(r0, n):
        idx = [(g, _rows(r0 + r, 16, 16)) for r in range(0, n, 16) for g in range(2)]
        return (lambda: [(wf_h[a].at[i], wf_v.at[(a,) + i]) for i in idx for a in range(3)],
                [wf_v.at[:, :, _rows(r0, n, 16)]])

    def wo(r0, n, g0, g1, step):
        idx = [(pl.ds(g, step), pl.ds(r0 + r, 16)) for r in range(0, n, 16) for g in range(g0, g1, step)]
        return (lambda: [(wo_h.at[i], wo_v.at[i]) for i in idx],
                [wo_v.at[pl.ds(g0, g1 - g0), pl.ds(r0, n)]])

    def wq_batch(b):
        return b, kv(1, b, HEADS_ALL), wq(b)

    def wf_batch(b):
        return 8 + b, kv(1, 8 + b, HEADS_ALL), wf(F0 + FB * b, FB)

    def k_batch(j):
        return EARLY + j, kv(0, j, HEADS_LONG), kv(0, j, HEADS_SHORT)

    def v_batch(j):
        return NT + j, kv(1, j, HEADS_LONG), kv(1, j, HEADS_SHORT)

    def wo_batch(b):
        return 2 * NT + b, wo(b * DH, DH, 0, 4, 4), wo(b * DH, DH, 4, 8, 2)

    def wait(batch):
        i, long_part, short_part = batch
        for sem, (_, regions) in ((sem_long, long_part), (sem_short, short_part)):
            for a in regions:
                pltpu.make_async_copy(a, a, sem.at[i % NSEM]).wait()

    def start_long(batch):
        for a, b in batch[1][0]():
            pltpu.make_async_copy(a, b, sem_long.at[batch[0] % NSEM]).start(priority=LONG)

    def start_short(copies, sem, pause, *work):
        at = {len(copies) * (i + 1) // (len(work) + 1): f for i, f in enumerate(work)}
        for i, (a, b) in enumerate(copies):
            if i in at:
                at[i]()
            pltpu.make_async_copy(a, b, sem).start(priority=SHORT)
            pl.delay(pause)

    def issue(batch, pause, *work):
        start_long(batch)
        start_short(batch[2][0](), sem_short.at[batch[0] % NSEM], pause, *work)

    tok = {}
    copy_x = pltpu.make_async_copy(x_h, x_v, sem_x.at[0])
    copy_wr = pltpu.make_async_copy(wr_h, wr_v, sem_x.at[1])

    def layernorm():
        copy_x.wait()
        copy_wr.wait()
        x = x_v[0].astype(F32)
        mean = jnp.mean(x, axis=-1, keepdims=True)
        var = jnp.mean(jnp.square(x - mean), axis=-1, keepdims=True)
        xn = ((x - mean) / jnp.sqrt(var + 1e-5)).astype(BF16)
        tok["xn"] = xn.astype(F32)
        tok["xn8"] = jnp.broadcast_to(xn, (8, D))
        tok["r"] = jnp.sum(tok["xn"] * wr_v[...].reshape(1, D).astype(F32), axis=-1, keepdims=True)
        g_v[0] = jnp.broadcast_to(x, (8, D))
        m_v[...] = jnp.full(m_v.shape, -jnp.inf, F32)
        l_v[...] = jnp.zeros(l_v.shape, F32)
        o_v[...] = jnp.zeros(o_v.shape, F32)

    def proj_q(s):
        w = wq_v[:, :, _rows(s * 8 * DH, 8 * DH, 8 * DH)].reshape(D, 8 * DH)
        q = jnp.dot(tok["xn8"], w, preferred_element_type=F32)
        q_v[s] = _per_head(lambda j: q[:, j * DH:(j + 1) * DH])

    def ffn(r0, n):
        g, u, d = (wf_v[a, :, pl.ds(r0, n)].reshape(2 * n, D) for a in range(3))
        gt = jax.lax.dot_general(tok["xn8"], g, _NT, preferred_element_type=F32)
        up = jax.lax.dot_general(tok["xn8"], u, _NT, preferred_element_type=F32)
        y = jnp.dot((jax.nn.silu(gt) * up).astype(BF16), d, preferred_element_type=F32)
        tok["y"] = tok.get("y", 0.0) + y

    def scores(c):
        for s in range(NS):
            q = q_v[s].astype(BF16)
            sc = _per_head(lambda j: jax.lax.dot_general(
                q, kv_v[0, 8 * s + j, _rows(c * DH, DH, DH)], _NT, preferred_element_type=F32))
            sc = sc * (DH ** -0.5)
            s_v[s, c] = sc
            m_v[s] = jnp.maximum(m_v[s], sc)

    def values(c):
        for s in range(NS):
            p = jnp.exp(s_v[s, c] - m_v[s])
            l_v[s] += p
            p = p.astype(BF16)
            o_v[s] += _per_head(lambda j: jnp.dot(
                p, kv_v[1, 8 * s + j, _rows(c * DH, DH, DH)], preferred_element_type=F32))

    def proj_o(b):
        row = jax.lax.broadcasted_iota(jnp.int32, (8, D), 0)
        for g in range(8):
            t = jnp.dot(o_v[g // 2].astype(BF16), wo_v[g, pl.ds(b * DH, DH)], preferred_element_type=F32)
            tok["attn"] = tok.get("attn", 0.0) + jnp.where(row == 4 * (g % 2) + b, t, 0.0)

    def proj_o_last(r, g0, n):
        for g in range(g0, g0 + n):
            coef = jnp.concatenate([c_v[g, pl.ds(r, 16)]] * (D // DH), axis=1)
            prod = wo_v[g, pl.ds(3 * DH + r, 16)].astype(F32) * coef
            tok["attn"] = tok["attn"] + (prod[0:8] + prod[8:16])

    opening, (opening_rows,) = wf(0, F0)
    start_long(wq_batch(0))
    start_short(opening(), sem_x.at[2], T_OPEN)
    copy_x.start(priority=SHORT)
    copy_wr.start(priority=SHORT)
    start_short(wq(0)[0](), sem_short.at[0], T_FIRST)
    issue(wq_batch(1), T_W, layernorm)
    wait(wq_batch(0))
    issue(wq_batch(2), T_W)

    @pl.loop(3, 8)
    def _(b):
        wait(wq_batch(b - 2))
        issue(wq_batch(b), T_W)

    @pl.loop(0, 2)
    def _(b):
        wait(wq_batch(6 + b))
        issue(wf_batch(b), T_W)

    @pl.loop(2, 8)
    def _(b):
        wait(wf_batch(b - 2))
        issue(wf_batch(b), T_Q, lambda: pl.when(b < 2 + NS)(lambda: proj_q(b - 2)))

    assert F0 + 8 * FB == FH
    pltpu.make_async_copy(opening_rows, opening_rows, sem_x.at[2]).wait()
    wait(wf_batch(6))
    issue(k_batch(0), T_F, lambda: ffn(0, 384))
    wait(wf_batch(7))
    issue(k_batch(1), T_F, lambda: ffn(384, FH - 384))
    upd = tok["xn"] * 0.0 + tok["y"] * jax.nn.sigmoid(tok["r"])
    g_v[1] = jax.nn.silu(tok["xn"] + upd)

    @pl.loop(2, NT)
    def _(j):
        wait(k_batch(j - 2))
        issue(k_batch(j), T_K, lambda: scores(j - 2))

    @pl.loop(0, 2)
    def _(j):
        wait(k_batch(NT - 2 + j))
        issue(v_batch(EARLY + j), T_K, lambda: scores(NT - 2 + j))

    for s in range(NS):
        m_v[s] = jnp.broadcast_to(jnp.max(m_v[s], axis=-1, keepdims=True), (8, DH))

    @pl.loop(EARLY + 2, NT)
    def _(j):
        wait(v_batch(j - 2))
        issue(v_batch(j), T_V, lambda: values(j - 2 - EARLY), lambda: values(j - 3))

    wait(v_batch(NT - 2))
    issue(wo_batch(0), T_VO, lambda: values(NT - 2 - EARLY), lambda: values(NT - 3))
    wait(v_batch(NT - 1))
    issue(wo_batch(1), T_VO, lambda: values(NT - 1), lambda: values(NT - 2))
    for s in range(NS):
        o = o_v[s] / jnp.sum(l_v[s], axis=-1, keepdims=True)
        o_v[s] = o.astype(BF16).astype(F32)

    tail, pos = [], 8
    for i, n in enumerate(TAIL):
        r, g0 = pos // 8 * 16, pos % 8
        idx = (pl.ds(g0, n), pl.ds(3 * DH + r, 16))
        tail.append((pltpu.make_async_copy(wo_h.at[idx], wo_v.at[idx], sem_tail.at[i]), r, g0, n))
        pos += n
    assert pos == 64
    last_batch = (2 * NT + 3, (lambda: [], []), wo(3 * DH, 16, 0, 8, 2))

    wait(wo_batch(0))
    start_long(wo_batch(2))
    for c, *_ in tail:
        c.start(priority=LONG)
    start_short(wo_batch(2)[2][0](), sem_short.at[(2 * NT + 2) % NSEM], T_O, lambda: proj_o(0))
    wait(wo_batch(1))
    issue(last_batch, T_O, lambda: proj_o(1))
    for g in range(8):
        j = 4 * (g % 2) + 3
        c_v[g] = jnp.broadcast_to(o_v[g // 2, j:j + 1], (DH, DH)).T
    wait(wo_batch(2))
    proj_o(2)
    wait(last_batch)
    proj_o_last(0, 0, 8)
    for c, r, g0, n in tail:
        c.wait()
        proj_o_last(r, g0, n)

    attn = jnp.sum(tok["attn"], axis=0, keepdims=True)
    res = g_v[0] + jnp.broadcast_to(attn, (8, D)) * g_v[1]
    out_ref[0] = res.astype(out_ref.dtype)[0:1]


@jax.jit
def pallas_recurrent_scan__sliding_block_cached__moe_arch_mod__decode_kernel(
    A_x: jax.Array,
    A_k_cache: jax.Array,
    A_v_cache: jax.Array,
    A_wq: jax.Array,
    A_wo: jax.Array,
    B_x: jax.Array,
    B_w_r: jax.Array,
    B_w_gate: jax.Array,
    B_w_up: jax.Array,
    B_w_down: jax.Array,
):
    del B_x
    hbm = pl.BlockSpec(memory_space=pltpu.HBM)
    dma = pltpu.SemaphoreType.DMA
    per_head = pltpu.VMEM((NS, 8, DH), F32)
    return pl.pallas_call(
        _kernel,
        out_shape=jax.ShapeDtypeStruct((1, 1, D), BF16),
        in_specs=[hbm] * 9,
        out_specs=pl.BlockSpec(memory_space=pltpu.VMEM),
        scratch_shapes=[
            pltpu.VMEM((1, 1, D), BF16),
            pltpu.VMEM((D,), BF16),
            pltpu.VMEM((8, D // 8, NH * DH), BF16),
            pltpu.VMEM((2, NH, W, DH), BF16),
            pltpu.VMEM((8, NH * DH // 8, D), BF16),
            pltpu.VMEM((3, 2, FH, D), BF16),
            per_head,
            pltpu.VMEM((NS, NT, 8, DH), F32),
            per_head, per_head, per_head,
            pltpu.VMEM((8, DH, DH), F32),
            pltpu.VMEM((2, 8, D), F32),
            dma((3,)), dma((NSEM,)), dma((NSEM,)), dma((len(TAIL),)),
        ],
        compiler_params=pltpu.CompilerParams(
            vmem_limit_bytes=100 * 1024 * 1024,
            disable_semaphore_checks=True,
        ),
    )(A_x, A_k_cache, A_v_cache, A_wq.reshape(8, D // 8, NH * DH), A_wo.reshape(8, NH * DH // 8, D), B_w_r,
      B_w_gate.T.reshape(2, FH, D), B_w_up.T.reshape(2, FH, D), B_w_down.reshape(2, FH, D))
```

```python
import jax
import jax.numpy as jnp
import jax.experimental.pallas as pl
import jax.experimental.pallas.tpu as pltpu

D = 512
NH = 32
DH = 128
SK = 32768
W = min(4096, max(256, SK // 4))
F = 1376

NT = W // DH
NS = NH // 8
RUN = 64
EARLY = 16
FH = F // 2
F0, FB = 48, 80
NSEM = 3
HEADS_ALL = (((0, 11),), ((11, 11),), ((22, 10),))
HEADS_LONG = (((0, 10),), ((10, 10),))
HEADS_SHORT = (((20, 2), (22, 2), (24, 2)), ((26, 2), (28, 2), (30, 2)))
TAIL = (8, 8, 8, 8, 8, 8, 4, 2, 1, 1)
T_OPEN, T_FIRST, T_W, T_Q, T_F, T_K, T_V, T_VO, T_O = 27, 30, 54, 47, 48, 58, 50, 46, 54

BF16 = jnp.bfloat16
F32 = jnp.float32
_NT = (((1,), (1,)), ((), ()))
LONG, SHORT = 1, 0


def _rows(start, size, align):
    return pl.ds(start if isinstance(start, int) else pl.multiple_of(start, align), size)


def _per_head(f):
    r = f(0)
    for j in range(1, 8):
        r = jnp.where(jax.lax.broadcasted_iota(jnp.int32, r.shape, 0) == j, f(j), r)
    return r


def _kernel(x_h, k_h, v_h, wq_h, wo_h, wr_h, wg_h, wu_h, wd_h, out_ref,
            x_v, wr_v, wq_v, kv_v, wo_v, wf_v, q_v, s_v, m_v, l_v, o_v, c_v, g_v,
            sem_x, sem_long, sem_short, sem_tail):
    kv_h = (k_h, v_h)
    wf_h = (wg_h, wu_h, wd_h)

    def kv(t, j, heads):
        r = (2 * j - t) * RUN
        wraps = isinstance(r, int) and r < 0
        runs = (r + W if wraps else r, r + RUN)
        hs = pl.ds(heads[0][0][0], sum(n for group in heads for _, n in group))
        return (lambda: [(kv_h[t].at[0, pl.ds(h, n), _rows(SK - W + r, RUN, RUN)],
                          kv_v.at[t, pl.ds(h, n), _rows(r, RUN, RUN)])
                         for group in heads for r in runs for h, n in group],
                [kv_v.at[t, pl.ds(h, n), pl.ds(r, RUN)] for group in heads for r in runs for h, n in group]
                if wraps else [kv_v.at[t, hs, _rows(r, 2 * RUN, RUN)]])

    def wq(b):
        rows = _rows(8 * b, 8, 8)
        idx = [(g0 + g, rows, pl.ds((c0 + c) * 8 * DH, 8 * DH))
               for c0 in (0, 2) for g0 in (0, 4) for c in range(2) for g in range(4)]
        return lambda: [(wq_h.at[i], wq_v.at[i]) for i in idx], [wq_v.at[:, rows]]

    def wf(r0, n):
        idx = [(g, _rows(r0 + r, 16, 16)) for r in range(0, n, 16) for g in range(2)]
        return (lambda: [(wf_h[a].at[i], wf_v.at[(a,) + i]) for i in idx for a in range(3)],
                [wf_v.at[:, :, _rows(r0, n, 16)]])

    def wo(r0, n, g0, g1, step):
        idx = [(pl.ds(g, step), pl.ds(r0 + r, 16)) for r in range(0, n, 16) for g in range(g0, g1, step)]
        return (lambda: [(wo_h.at[i], wo_v.at[i]) for i in idx],
                [wo_v.at[pl.ds(g0, g1 - g0), pl.ds(r0, n)]])

    def wq_batch(b):
        return b, kv(1, b, HEADS_ALL), wq(b)

    def wf_batch(b):
        return 8 + b, kv(1, 8 + b, HEADS_ALL), wf(F0 + FB * b, FB)

    def k_batch(j):
        return EARLY + j, kv(0, j, HEADS_LONG), kv(0, j, HEADS_SHORT)

    def v_batch(j):
        return NT + j, kv(1, j, HEADS_LONG), kv(1, j, HEADS_SHORT)

    def wo_batch(b):
        return 2 * NT + b, wo(b * DH, DH, 0, 4, 4), wo(b * DH, DH, 4, 8, 2)

    def wait(batch):
        i, long_part, short_part = batch
        for sem, (_, regions) in ((sem_long, long_part), (sem_short, short_part)):
            for a in regions:
                pltpu.make_async_copy(a, a, sem.at[i % NSEM]).wait()

    def start_long(batch):
        for a, b in batch[1][0]():
            pltpu.make_async_copy(a, b, sem_long.at[batch[0] % NSEM]).start(priority=LONG)

    def start_short(copies, sem, pause, *work):
        at = {len(copies) * (i + 1) // (len(work) + 1): f for i, f in enumerate(work)}
        for i, (a, b) in enumerate(copies):
            if i in at:
                at[i]()
            pltpu.make_async_copy(a, b, sem).start(priority=SHORT)
            pl.delay(pause)

    def issue(batch, pause, *work):
        start_long(batch)
        start_short(batch[2][0](), sem_short.at[batch[0] % NSEM], pause, *work)

    tok = {}
    copy_x = pltpu.make_async_copy(x_h, x_v, sem_x.at[0])
    copy_wr = pltpu.make_async_copy(wr_h, wr_v, sem_x.at[1])

    def layernorm():
        copy_x.wait()
        copy_wr.wait()
        x = x_v[0].astype(F32)
        mean = jnp.mean(x, axis=-1, keepdims=True)
        var = jnp.mean(jnp.square(x - mean), axis=-1, keepdims=True)
        xn = ((x - mean) / jnp.sqrt(var + 1e-5)).astype(BF16)
        tok["xn"] = xn.astype(F32)
        tok["xn8"] = jnp.broadcast_to(xn, (8, D))
        tok["r"] = jnp.sum(tok["xn"] * wr_v[...].reshape(1, D).astype(F32), axis=-1, keepdims=True)
        g_v[0] = jnp.broadcast_to(x, (8, D))
        m_v[...] = jnp.full(m_v.shape, -jnp.inf, F32)
        l_v[...] = jnp.zeros(l_v.shape, F32)
        o_v[...] = jnp.zeros(o_v.shape, F32)

    def proj_q(s):
        w = wq_v[:, :, _rows(s * 8 * DH, 8 * DH, 8 * DH)].reshape(D, 8 * DH)
        q = jnp.dot(tok["xn8"], w, preferred_element_type=F32)
        q_v[s] = _per_head(lambda j: q[:, j * DH:(j + 1) * DH])

    def ffn(r0, n):
        g, u, d = (wf_v[a, :, pl.ds(r0, n)].reshape(2 * n, D) for a in range(3))
        gt = jax.lax.dot_general(tok["xn8"], g, _NT, preferred_element_type=F32)
        up = jax.lax.dot_general(tok["xn8"], u, _NT, preferred_element_type=F32)
        y = jnp.dot((jax.nn.silu(gt) * up).astype(BF16), d, preferred_element_type=F32)
        tok["y"] = tok.get("y", 0.0) + y

    def scores(c):
        for s in range(NS):
            q = q_v[s].astype(BF16)
            sc = _per_head(lambda j: jax.lax.dot_general(
                q, kv_v[0, 8 * s + j, _rows(c * DH, DH, DH)], _NT, preferred_element_type=F32))
            sc = sc * (DH ** -0.5)
            s_v[s, c] = sc
            m_v[s] = jnp.maximum(m_v[s], sc)

    def values(c):
        for s in range(NS):
            p = jnp.exp(s_v[s, c] - m_v[s])
            l_v[s] += p
            p = p.astype(BF16)
            o_v[s] += _per_head(lambda j: jnp.dot(
                p, kv_v[1, 8 * s + j, _rows(c * DH, DH, DH)], preferred_element_type=F32))

    def proj_o(b):
        row = jax.lax.broadcasted_iota(jnp.int32, (8, D), 0)
        for g in range(8):
            t = jnp.dot(o_v[g // 2].astype(BF16), wo_v[g, pl.ds(b * DH, DH)], preferred_element_type=F32)
            tok["attn"] = tok.get("attn", 0.0) + jnp.where(row == 4 * (g % 2) + b, t, 0.0)

    def proj_o_last(r, g0, n):
        for g in range(g0, g0 + n):
            coef = jnp.concatenate([c_v[g, pl.ds(r, 16)]] * (D // DH), axis=1)
            prod = wo_v[g, pl.ds(3 * DH + r, 16)].astype(F32) * coef
            tok["attn"] = tok["attn"] + (prod[0:8] + prod[8:16])

    opening, (opening_rows,) = wf(0, F0)
    start_long(wq_batch(0))
    start_short(opening(), sem_x.at[2], T_OPEN)
    copy_x.start(priority=SHORT)
    copy_wr.start(priority=SHORT)
    start_short(wq(0)[0](), sem_short.at[0], T_FIRST)
    issue(wq_batch(1), T_W, layernorm)
    for b in range(2, 10):
        wait(wq_batch(b - 2))
        issue(wq_batch(b) if b < 8 else wf_batch(b - 8), T_W)
    for s in range(NS):
        wait(wf_batch(s))
        issue(wf_batch(s + 2), T_Q, lambda: proj_q(s))
    assert F0 + 8 * FB == FH
    pltpu.make_async_copy(opening_rows, opening_rows, sem_x.at[2]).wait()
    for b, (r0, n) in enumerate(((0, 192), (192, 192), (384, 128), (512, FH - 512))):
        wait(wf_batch(4 + b))
        issue(wf_batch(6 + b) if b < 2 else k_batch(b - 2), T_F, lambda: ffn(r0, n))
    upd = tok["xn"] * 0.0 + tok["y"] * jax.nn.sigmoid(tok["r"])
    g_v[1] = jax.nn.silu(tok["xn"] + upd)

    @pl.loop(2, NT)
    def _(j):
        wait(k_batch(j - 2))
        issue(k_batch(j), T_K, lambda: scores(j - 2))

    @pl.loop(0, 2)
    def _(j):
        wait(k_batch(NT - 2 + j))
        issue(v_batch(EARLY + j), T_K, lambda: scores(NT - 2 + j))

    for s in range(NS):
        m_v[s] = jnp.broadcast_to(jnp.max(m_v[s], axis=-1, keepdims=True), (8, DH))

    @pl.loop(EARLY + 2, NT)
    def _(j):
        wait(v_batch(j - 2))
        issue(v_batch(j), T_V, lambda: values(j - 2 - EARLY), lambda: values(j - 3))

    wait(v_batch(NT - 2))
    issue(wo_batch(0), T_VO, lambda: values(NT - 2 - EARLY), lambda: values(NT - 3))
    wait(v_batch(NT - 1))
    issue(wo_batch(1), T_VO, lambda: values(NT - 1), lambda: values(NT - 2))
    for s in range(NS):
        o = o_v[s] / jnp.sum(l_v[s], axis=-1, keepdims=True)
        o_v[s] = o.astype(BF16).astype(F32)

    tail, pos = [], 8
    for i, n in enumerate(TAIL):
        r, g0 = pos // 8 * 16, pos % 8
        idx = (pl.ds(g0, n), pl.ds(3 * DH + r, 16))
        tail.append((pltpu.make_async_copy(wo_h.at[idx], wo_v.at[idx], sem_tail.at[i]), r, g0, n))
        pos += n
    assert pos == 64
    last_batch = (2 * NT + 3, (lambda: [], []), wo(3 * DH, 16, 0, 8, 2))

    wait(wo_batch(0))
    start_long(wo_batch(2))
    for c, *_ in tail:
        c.start(priority=LONG)
    start_short(wo_batch(2)[2][0](), sem_short.at[(2 * NT + 2) % NSEM], T_O, lambda: proj_o(0))
    wait(wo_batch(1))
    issue(last_batch, T_O, lambda: proj_o(1))
    for g in range(8):
        j = 4 * (g % 2) + 3
        c_v[g] = jnp.broadcast_to(o_v[g // 2, j:j + 1], (DH, DH)).T
    wait(wo_batch(2))
    proj_o(2)
    wait(last_batch)
    proj_o_last(0, 0, 8)
    for c, r, g0, n in tail:
        c.wait()
        proj_o_last(r, g0, n)

    attn = jnp.sum(tok["attn"], axis=0, keepdims=True)
    res = g_v[0] + jnp.broadcast_to(attn, (8, D)) * g_v[1]
    out_ref[0] = res.astype(out_ref.dtype)[0:1]


@jax.jit
def pallas_recurrent_scan__sliding_block_cached__moe_arch_mod__decode_kernel(
    A_x: jax.Array,
    A_k_cache: jax.Array,
    A_v_cache: jax.Array,
    A_wq: jax.Array,
    A_wo: jax.Array,
    B_x: jax.Array,
    B_w_r: jax.Array,
    B_w_gate: jax.Array,
    B_w_up: jax.Array,
    B_w_down: jax.Array,
):
    del B_x
    hbm = pl.BlockSpec(memory_space=pltpu.HBM)
    dma = pltpu.SemaphoreType.DMA
    per_head = pltpu.VMEM((NS, 8, DH), F32)
    return pl.pallas_call(
        _kernel,
        out_shape=jax.ShapeDtypeStruct((1, 1, D), BF16),
        in_specs=[hbm] * 9,
        out_specs=pl.BlockSpec(memory_space=pltpu.VMEM),
        scratch_shapes=[
            pltpu.VMEM((1, 1, D), BF16),
            pltpu.VMEM((D,), BF16),
            pltpu.VMEM((8, D // 8, NH * DH), BF16),
            pltpu.VMEM((2, NH, W, DH), BF16),
            pltpu.VMEM((8, NH * DH // 8, D), BF16),
            pltpu.VMEM((3, 2, FH, D), BF16),
            per_head,
            pltpu.VMEM((NS, NT, 8, DH), F32),
            per_head, per_head, per_head,
            pltpu.VMEM((8, DH, DH), F32),
            pltpu.VMEM((2, 8, D), F32),
            dma((3,)), dma((NSEM,)), dma((NSEM,)), dma((len(TAIL),)),
        ],
        compiler_params=pltpu.CompilerParams(
            vmem_limit_bytes=100 * 1024 * 1024,
            disable_semaphore_checks=True,
        ),
    )(A_x, A_k_cache, A_v_cache, A_wq.reshape(8, D // 8, NH * DH), A_wo.reshape(8, NH * DH // 8, D), B_w_r,
      B_w_gate.T.reshape(2, FH, D), B_w_up.T.reshape(2, FH, D), B_w_down.reshape(2, FH, D))
```

```python
import jax
import jax.numpy as jnp
import jax.experimental.pallas as pl
import jax.experimental.pallas.tpu as pltpu

D = 512
NH = 32
DH = 128
SK = 32768
W = min(4096, max(256, SK // 4))
F = 1376

NT = W // DH
NS = NH // 8
RUN = 64
EARLY = 16
FH = F // 2
F0, FB = 48, 80
NSEM = 3
HEADS_ALL = ((0, 8, 0), (0, 16, 1), (8, 16, 0), (16, 16, 1), (24, 8, 0))
HEADS_LONG = ((0, 10, 0), (0, 10, 1), (10, 10, 0), (10, 10, 1))
HEADS_SHORT = tuple((h + g, 2, i) for h in (20, 26) for i in (0, 1) for g in (0, 2, 4))
TAIL = (8, 8, 8, 8, 8, 8, 4, 2, 1, 1)
T_OPEN, T_FIRST, T_W, T_Q, T_F, T_K, T_V, T_VO, T_O = 27, 30, 54, 50, 50, 61, 50, 48, 54

BF16 = jnp.bfloat16
F32 = jnp.float32
_NT = (((1,), (1,)), ((), ()))
LONG, SHORT = 1, 0


def _rows(start, size, align):
    return pl.ds(start if isinstance(start, int) else pl.multiple_of(start, align), size)


def _per_head(f):
    r = f(0)
    for j in range(1, 8):
        r = jnp.where(jax.lax.broadcasted_iota(jnp.int32, r.shape, 0) == j, f(j), r)
    return r


def _kernel(x_h, k_h, v_h, wq_h, wo_h, wr_h, wg_h, wu_h, wd_h, out_ref,
            x_v, wr_v, wq_v, kv_v, wo_v, wf_v, q_v, s_v, m_v, l_v, o_v, c_v, g_v,
            sem_x, sem_long, sem_short, sem_tail):
    kv_h = (k_h, v_h)
    wf_h = (wg_h, wu_h, wd_h)

    def kv(t, j, heads):
        r = (2 * j - t) * RUN
        wraps = isinstance(r, int) and r < 0
        runs = (r + W if wraps else r, r + RUN)
        hs = pl.ds(min(heads)[0], sum(n for _, n, _ in heads) // 2)
        return (lambda: [(kv_h[t].at[0, pl.ds(h, n), _rows(SK - W + runs[i], RUN, RUN)],
                          kv_v.at[t, pl.ds(h, n), _rows(runs[i], RUN, RUN)]) for h, n, i in heads],
                [kv_v.at[t, pl.ds(h, n), pl.ds(runs[i], RUN)] for h, n, i in heads] if wraps
                else [kv_v.at[t, hs, _rows(r, 2 * RUN, RUN)]])

    def wq(b):
        rows = _rows(8 * b, 8, 8)
        idx = [(g0 + g, rows, pl.ds((c0 + c) * 8 * DH, 8 * DH))
               for c0 in (0, 2) for g0 in (0, 1, 4, 5) for c in range(2) for g in (0, 2)]
        return lambda: [(wq_h.at[i], wq_v.at[i]) for i in idx], [wq_v.at[:, rows]]

    def wf(r0, n):
        idx = [(g, _rows(r0 + r, 16, 16)) for r in range(0, n, 16) for g in range(2)]
        return (lambda: [(wf_h[a].at[i], wf_v.at[(a,) + i]) for i in idx for a in range(3)],
                [wf_v.at[:, :, _rows(r0, n, 16)]])

    def wo(r0, n, g0, g1, step):
        idx = [(pl.ds(g, step), pl.ds(r0 + r, 16)) for r in range(0, n, 16) for g in range(g0, g1, step)]
        return (lambda: [(wo_h.at[i], wo_v.at[i]) for i in idx],
                [wo_v.at[pl.ds(g0, g1 - g0), pl.ds(r0, n)]])

    def wq_batch(b):
        return b, kv(1, b, HEADS_ALL), wq(b)

    def wf_batch(b):
        return 8 + b, kv(1, 8 + b, HEADS_ALL), wf(F0 + FB * b, FB)

    def k_batch(j):
        return EARLY + j, kv(0, j, HEADS_LONG), kv(0, j, HEADS_SHORT)

    def v_batch(j):
        return NT + j, kv(1, j, HEADS_LONG), kv(1, j, HEADS_SHORT)

    def wo_batch(b):
        return 2 * NT + b, wo(b * DH, DH, 0, 4, 4), wo(b * DH, DH, 4, 8, 2)

    def wait(batch):
        i, long_part, short_part = batch
        for sem, (_, regions) in ((sem_long, long_part), (sem_short, short_part)):
            for a in regions:
                pltpu.make_async_copy(a, a, sem.at[i % NSEM]).wait()

    def start_long(batch):
        for a, b in batch[1][0]():
            pltpu.make_async_copy(a, b, sem_long.at[batch[0] % NSEM]).start(priority=LONG)

    def start_short(copies, sem, pause, *work):
        at = {len(copies) * (i + 1) // (len(work) + 1): f for i, f in enumerate(work)}
        for i, (a, b) in enumerate(copies):
            if i in at:
                at[i]()
            pltpu.make_async_copy(a, b, sem).start(priority=SHORT)
            pl.delay(pause)

    def issue(batch, pause, *work):
        start_long(batch)
        start_short(batch[2][0](), sem_short.at[batch[0] % NSEM], pause, *work)

    tok = {}
    copy_x = pltpu.make_async_copy(x_h, x_v, sem_x.at[0])
    copy_wr = pltpu.make_async_copy(wr_h, wr_v, sem_x.at[1])

    def layernorm():
        copy_x.wait()
        copy_wr.wait()
        x = x_v[0].astype(F32)
        mean = jnp.mean(x, axis=-1, keepdims=True)
        var = jnp.mean(jnp.square(x - mean), axis=-1, keepdims=True)
        xn = ((x - mean) / jnp.sqrt(var + 1e-5)).astype(BF16)
        tok["xn"] = xn.astype(F32)
        tok["xn8"] = jnp.broadcast_to(xn, (8, D))
        tok["r"] = jnp.sum(tok["xn"] * wr_v[...].reshape(1, D).astype(F32), axis=-1, keepdims=True)
        g_v[0] = jnp.broadcast_to(x, (8, D))
        m_v[...] = jnp.full(m_v.shape, -jnp.inf, F32)
        l_v[...] = jnp.zeros(l_v.shape, F32)
        o_v[...] = jnp.zeros(o_v.shape, F32)

    def proj_q(s):
        w = wq_v[:, :, _rows(s * 8 * DH, 8 * DH, 8 * DH)].reshape(D, 8 * DH)
        q = jnp.dot(tok["xn8"], w, preferred_element_type=F32)
        q_v[s] = _per_head(lambda j: q[:, j * DH:(j + 1) * DH])

    def ffn(r0, n):
        g, u, d = (wf_v[a, :, pl.ds(r0, n)].reshape(2 * n, D) for a in range(3))
        gt = jax.lax.dot_general(tok["xn8"], g, _NT, preferred_element_type=F32)
        up = jax.lax.dot_general(tok["xn8"], u, _NT, preferred_element_type=F32)
        y = jnp.dot((jax.nn.silu(gt) * up).astype(BF16), d, preferred_element_type=F32)
        tok["y"] = tok.get("y", 0.0) + y

    def scores(c):
        for s in range(NS):
            q = q_v[s].astype(BF16)
            sc = _per_head(lambda j: jax.lax.dot_general(
                q, kv_v[0, 8 * s + j, _rows(c * DH, DH, DH)], _NT, preferred_element_type=F32))
            sc = sc * (DH ** -0.5)
            s_v[s, c] = sc
            m_v[s] = jnp.maximum(m_v[s], sc)

    def values(c):
        for s in range(NS):
            p = jnp.exp(s_v[s, c] - m_v[s])
            l_v[s] += p
            p = p.astype(BF16)
            o_v[s] += _per_head(lambda j: jnp.dot(
                p, kv_v[1, 8 * s + j, _rows(c * DH, DH, DH)], preferred_element_type=F32))

    def proj_o(b):
        row = jax.lax.broadcasted_iota(jnp.int32, (8, D), 0)
        for g in range(8):
            t = jnp.dot(o_v[g // 2].astype(BF16), wo_v[g, pl.ds(b * DH, DH)], preferred_element_type=F32)
            tok["attn"] = tok.get("attn", 0.0) + jnp.where(row == 4 * (g % 2) + b, t, 0.0)

    def proj_o_last(r, g0, n):
        for g in range(g0, g0 + n):
            coef = jnp.concatenate([c_v[g, pl.ds(r, 16)]] * (D // DH), axis=1)
            prod = wo_v[g, pl.ds(3 * DH + r, 16)].astype(F32) * coef
            tok["attn"] = tok["attn"] + (prod[0:8] + prod[8:16])

    opening, (opening_rows,) = wf(0, F0)
    start_long(wq_batch(0))
    start_short(opening(), sem_x.at[2], T_OPEN)
    copy_x.start(priority=SHORT)
    copy_wr.start(priority=SHORT)
    start_short(wq(0)[0](), sem_short.at[0], T_FIRST)
    issue(wq_batch(1), T_W, layernorm)
    for b in range(2, 10):
        wait(wq_batch(b - 2))
        issue(wq_batch(b) if b < 8 else wf_batch(b - 8), T_W)
    for s in range(NS):
        wait(wf_batch(s))
        issue(wf_batch(s + 2), T_Q, lambda: proj_q(s))
    assert F0 + 8 * FB == FH
    pltpu.make_async_copy(opening_rows, opening_rows, sem_x.at[2]).wait()
    for b, (r0, n) in enumerate(((0, 192), (192, 192), (384, 128), (512, FH - 512))):
        wait(wf_batch(4 + b))
        issue(wf_batch(6 + b) if b < 2 else k_batch(b - 2), T_F, lambda: ffn(r0, n))
    upd = tok["xn"] * 0.0 + tok["y"] * jax.nn.sigmoid(tok["r"])
    g_v[1] = jax.nn.silu(tok["xn"] + upd)

    @pl.loop(2, NT)
    def _(j):
        wait(k_batch(j - 2))
        issue(k_batch(j), T_K, lambda: scores(j - 2))

    @pl.loop(0, 2)
    def _(j):
        wait(k_batch(NT - 2 + j))
        issue(v_batch(EARLY + j), T_K, lambda: scores(NT - 2 + j))

    for s in range(NS):
        m_v[s] = jnp.broadcast_to(jnp.max(m_v[s], axis=-1, keepdims=True), (8, DH))

    @pl.loop(EARLY + 2, NT)
    def _(j):
        wait(v_batch(j - 2))
        issue(v_batch(j), T_V, lambda: values(j - 2 - EARLY), lambda: values(j - 3))

    wait(v_batch(NT - 2))
    issue(wo_batch(0), T_VO, lambda: values(NT - 2 - EARLY), lambda: values(NT - 3))
    wait(v_batch(NT - 1))
    issue(wo_batch(1), T_VO, lambda: values(NT - 1), lambda: values(NT - 2))
    for s in range(NS):
        o = o_v[s] / jnp.sum(l_v[s], axis=-1, keepdims=True)
        o_v[s] = o.astype(BF16).astype(F32)

    tail, pos = [], 8
    for i, n in enumerate(TAIL):
        r, g0 = pos // 8 * 16, pos % 8
        idx = (pl.ds(g0, n), pl.ds(3 * DH + r, 16))
        tail.append((pltpu.make_async_copy(wo_h.at[idx], wo_v.at[idx], sem_tail.at[i]), r, g0, n))
        pos += n
    assert pos == 64
    last_batch = (2 * NT + 3, (lambda: [], []), wo(3 * DH, 16, 0, 8, 2))

    wait(wo_batch(0))
    start_long(wo_batch(2))
    for c, *_ in tail:
        c.start(priority=LONG)
    start_short(wo_batch(2)[2][0](), sem_short.at[(2 * NT + 2) % NSEM], T_O, lambda: proj_o(0))
    wait(wo_batch(1))
    issue(last_batch, T_O, lambda: proj_o(1))
    for g in range(8):
        j = 4 * (g % 2) + 3
        c_v[g] = jnp.broadcast_to(o_v[g // 2, j:j + 1], (DH, DH)).T
    wait(wo_batch(2))
    proj_o(2)
    wait(last_batch)
    proj_o_last(0, 0, 8)
    for c, r, g0, n in tail:
        c.wait()
        proj_o_last(r, g0, n)

    attn = jnp.sum(tok["attn"], axis=0, keepdims=True)
    res = g_v[0] + jnp.broadcast_to(attn, (8, D)) * g_v[1]
    out_ref[0] = res.astype(out_ref.dtype)[0:1]


@jax.jit
def pallas_recurrent_scan__sliding_block_cached__moe_arch_mod__decode_kernel(
    A_x: jax.Array,
    A_k_cache: jax.Array,
    A_v_cache: jax.Array,
    A_wq: jax.Array,
    A_wo: jax.Array,
    B_x: jax.Array,
    B_w_r: jax.Array,
    B_w_gate: jax.Array,
    B_w_up: jax.Array,
    B_w_down: jax.Array,
):
    del B_x
    hbm = pl.BlockSpec(memory_space=pltpu.HBM)
    dma = pltpu.SemaphoreType.DMA
    per_head = pltpu.VMEM((NS, 8, DH), F32)
    return pl.pallas_call(
        _kernel,
        out_shape=jax.ShapeDtypeStruct((1, 1, D), BF16),
        in_specs=[hbm] * 9,
        out_specs=pl.BlockSpec(memory_space=pltpu.VMEM),
        scratch_shapes=[
            pltpu.VMEM((1, 1, D), BF16),
            pltpu.VMEM((D,), BF16),
            pltpu.VMEM((8, D // 8, NH * DH), BF16),
            pltpu.VMEM((2, NH, W, DH), BF16),
            pltpu.VMEM((8, NH * DH // 8, D), BF16),
            pltpu.VMEM((3, 2, FH, D), BF16),
            per_head,
            pltpu.VMEM((NS, NT, 8, DH), F32),
            per_head, per_head, per_head,
            pltpu.VMEM((8, DH, DH), F32),
            pltpu.VMEM((2, 8, D), F32),
            dma((3,)), dma((NSEM,)), dma((NSEM,)), dma((len(TAIL),)),
        ],
        compiler_params=pltpu.CompilerParams(
            vmem_limit_bytes=100 * 1024 * 1024,
            disable_semaphore_checks=True,
        ),
    )(A_x, A_k_cache, A_v_cache, A_wq.reshape(8, D // 8, NH * DH), A_wo.reshape(8, NH * DH // 8, D), B_w_r,
      B_w_gate.T.reshape(2, FH, D), B_w_up.T.reshape(2, FH, D), B_w_down.reshape(2, FH, D))
```
